```python
import jax
import jax.numpy as jnp

def _softmax(x, axis=-1):
    return jax.nn.softmax(x, axis=axis)
def _gelu(x):
    return jax.nn.gelu(x, approximate=True)
def _silu(x):
    return jax.nn.silu(x)
def _sigmoid(x):
    return jax.nn.sigmoid(x)
def _layernorm(x, axis=-1, eps=1e-5):
    m = jnp.mean(x, axis=axis, keepdims=True)
    v = jnp.var(x, axis=axis, keepdims=True)
    return (x - m) / jnp.sqrt(v + eps)
def _scatter_add(tgt, idx, src, axis=0):
    return tgt.at[idx].add(src)
def _segment_sum(src, seg, n):
    return jax.ops.segment_sum(src, seg, n)
class _Rng:
    def __init__(self, key):
        self._k = key
    def _next(self):
        self._k, sub = jax.random.split(self._k)
        return sub
    def normal(self, shape):
        return jax.random.normal(self._next(), shape, dtype=jnp.bfloat16)
    def randint(self, lo, hi, shape):
        return jax.random.randint(self._next(), shape, lo, hi, dtype=jnp.int32)
    def uniform(self, shape, lo=0.0, hi=1.0):
        return jax.random.uniform(self._next(), shape, jnp.bfloat16, lo, hi)
    def permutation(self, n):
        return jax.random.permutation(self._next(), n)


kernel_name = 'standalone__batchnorm__sampling'

def setup_inputs():
    _rng = _Rng(jax.random.key(int.from_bytes(__import__("os").urandom(4), "little")))
    _w = (lambda a: (lambda t: t.astype(jnp.bfloat16) if jnp.issubdtype(t.dtype, jnp.floating) else t)(jnp.asarray(a)))
    B, S, C = 1024, 32, 576
    K = 3
    return {
        "x": _w((lambda *s: _rng.normal(s) * 0.05)(B, S, C)),
        "w": _w((lambda *s: _rng.normal(s) * 0.05)(K, C, C) * (1.0 / (K * C) ** 0.5)),
        "mean": _w((lambda *s: _rng.normal(s) * 0.05)(C) * 0.1),
        "var": _w(jnp.abs((lambda *s: _rng.normal(s) * 0.05)(C)) + 0.5),
        "g": _w((lambda *s: _rng.normal(s) * 0.05)(C) + 1.0),
        "b": _w((lambda *s: _rng.normal(s) * 0.05)(C) * 0.1),
    }

def reference(x, w, mean, var, g, b):
    K = 3
    P = K // 2
    S = x.shape[1]
    xp = jnp.pad(x, ((0, 0), (P, P), (0, 0)))
    y = sum(jnp.einsum('bsc,cd->bsd', xp[:, k:k + S, :], w[k]) for k in range(K))
    inv_std = 1.0 / jnp.sqrt(var + 1e-5)
    y = (y - mean) * (g * inv_std) + b
    return _silu(y)
```

```python
import jax
import jax.numpy as jnp
from jax.experimental import pallas as pl
from jax.experimental.pallas import tpu as pltpu

def make(p=0.5, q=2.0, D=3, RX=8, RO=4, act='tanh', fold=True, sep=True, flags=None, ktl=True, U=1):
  p2=p*p; q2=q*q
  N0 = p2*q2; Np = 2*p2*(p2-q2); Nq = 2*q2*(q2-p2)
  def f(x, w, mean, var, g, b):
    B, S, C = x.shape
    NT = B // 128; NJ = S // 4; T = NT * NJ
    KT = (C + 127) // 128
    xt = jnp.transpose(x, (1, 2, 0))
    def kernel(x_hbm, w_hbm, mean_ref, var_ref, g_ref, b_ref, o_hbm,
               wbuf, xbuf, obuf, u_ref, sc_ref, sh_ref, sem_w, sem_x, sem_o, flag_ref):
        def x_dma(t):
            n = t >> 3; j = t & 7
            return pltpu.make_async_copy(x_hbm.at[pl.ds(4*j, 4), :, pl.ds(pl.multiple_of(n*128, 128), 128)], xbuf.at[t & (RX-1)], sem_x.at[t & (RX-1)])
        def o_dma(t):
            n = t >> 3; j = t & 7
            return pltpu.make_async_copy(obuf.at[t & (RO-1)], o_hbm.at[pl.ds(4*j, 4), :, pl.ds(pl.multiple_of(n*128, 128), 128)], sem_o.at[t & (RO-1)])
        wd = pltpu.make_async_copy(w_hbm, wbuf, sem_w.at[0])
        wd.start()
        flag_ref[0] = 0
        for t in range(1 + D):
            x_dma(t).start()
        xbuf[RX - 1, 3] = jnp.zeros((C, 128), jnp.bfloat16)
        inv = jax.lax.rsqrt(var_ref[...].astype(jnp.float32) + 1e-5)
        sc = (g_ref[...].astype(jnp.float32) * inv).reshape(1, C)
        sh = b_ref[...].astype(jnp.float32).reshape(1, C) - mean_ref[...].astype(jnp.float32).reshape(1, C) * sc
        if act == 'tanh':
            sc = sc * 0.5; sh = sh * 0.5
        if not fold:
            sc_ref[...] = jnp.broadcast_to(sc, (128, C)).T
        sh_ref[...] = jnp.broadcast_to(sh, (128, C)).T
        wd.wait()
        ws = [wbuf[k].astype(jnp.float32) for k in range(3)]
        if fold:
            ws = [a * sc for a in ws]
        w0, w1, w2 = [a.T for a in ws]
        us = [w0 * (1.0/N0), (w0 + p2*w2 + p*w1) * (1.0/Np), (w0 + p2*w2 - p*w1) * (1.0/Np),
              (w0 + q2*w2 + q*w1) * (1.0/Nq), (w0 + q2*w2 - q*w1) * (1.0/Nq), w2]
        for i in range(6):
            ub = us[i].astype(jnp.bfloat16)
            if ktl:
                for kt in range(KT):
                    wk = min(128, C - kt*128)
                    u_ref[i, kt, :, :wk] = ub[:, kt*128:kt*128+wk]
            else:
                u_ref[i] = ub
        x_dma(0).wait()

        def compute(t):
            j = t & 7
            cur = t & (RX-1)
            ld = lambda slot, i: xbuf[slot, i].astype(jnp.float32)
            d1 = ld(cur, 0); d2 = ld(cur, 1); d3 = ld(cur, 2); d4 = ld(cur, 3)
            d0 = jnp.where(j > 0, ld((t + RX - 1) & (RX-1), 3), 0.0)
            d5 = jnp.where(j < NJ - 1, ld((t + 1) & (RX-1), 0), 0.0)
            def dot(i, e):
                if ktl:
                    lhs = jnp.concatenate([u_ref[i, kt] for kt in range(KT - 1)] + [u_ref[i, KT-1][:, :C - (KT-1)*128]], axis=1)
                else:
                    lhs = u_ref[i]
                return jnp.dot(lhs, e.astype(jnp.bfloat16), preferred_element_type=jnp.float32)
            shv = sh_ref[...]
            scv = None if fold else sc_ref[...]
            def fin(i, y):
                z = y + shv if fold else y * scv + shv
                if act == 'tanh':
                    o = z * jnp.tanh(z) + z
                else:
                    o = z * pl.reciprocal(1.0 + jnp.exp(-z), approx=True)
                obuf[t & (RO-1), i] = o.astype(jnp.bfloat16)
            A = d4 - q2*d2; Bq = p * (d3 - q2*d1)
            m1 = dot(1, A + Bq)
            m2 = dot(2, A - Bq)
            s1 = m1 + m2; t1 = m1 - m2
            Cc = d4 - p2*d2; Dq = q * (d3 - p2*d1)
            m3 = dot(3, Cc + Dq)
            m4 = dot(4, Cc - Dq)
            s2 = m3 + m4; t2 = m3 - m4
            m0 = dot(0, N0*d0 - (p2+q2)*d2 + d4)
            fin(1, p*t1 + q*t2)
            fin(2, p2*s1 + q2*s2)
            m5 = dot(5, N0*d1 - (p2+q2)*d3 + d5)
            fin(0, m0 + s1 + s2)
            fin(3, p2*p*t1 + q2*q*t2 + m5)

        def body(it, _):
            t0 = it * U
            for k in range(U):
                t = t0 + k
                @pl.when(t + 1 < T)
                def _():
                    sl = (t + 1) & (RX - 1)
                    pltpu.make_async_copy(xbuf.at[sl], xbuf.at[sl], sem_x.at[sl]).wait()
                @pl.when(t >= RO)
                def _():
                    sl = t & (RO - 1)
                    pltpu.make_async_copy(obuf.at[sl], obuf.at[sl], sem_o.at[sl]).wait()
            for k in range(U):
                compute(t0 + k)
                t = t0 + k
                o_dma(t).start()
                @pl.when(t + 1 + D < T)
                def _():
                    x_dma(t + 1 + D).start()
            return 0
        jax.lax.fori_loop(0, T // U, body, 0)
        for t in range(T - RO, T):
            o_dma(t).wait()

    vm = pl.BlockSpec(memory_space=pltpu.VMEM)
    out = pl.pallas_call(
        kernel,
        in_specs=[pl.BlockSpec(memory_space=pl.ANY), pl.BlockSpec(memory_space=pl.ANY), vm, vm, vm, vm],
        out_specs=pl.BlockSpec(memory_space=pl.ANY),
        out_shape=jax.ShapeDtypeStruct((S, C, B), x.dtype),
        scratch_shapes=[pltpu.VMEM((3, C, C), jnp.bfloat16),
                        pltpu.VMEM((RX, 4, C, 128), jnp.bfloat16),
                        pltpu.VMEM((RO, 4, C, 128), jnp.bfloat16),
                        pltpu.VMEM((6, KT, C, 128) if ktl else (6, C, C), jnp.bfloat16),
                        pltpu.VMEM((C, 128), jnp.float32), pltpu.VMEM((C, 128), jnp.float32),
                        pltpu.SemaphoreType.DMA((1,)), pltpu.SemaphoreType.DMA((RX,)), pltpu.SemaphoreType.DMA((RO,)),
                        pltpu.SMEM((1,), jnp.int32)],
        compiler_params=pltpu.CompilerParams(vmem_limit_bytes=64*1024*1024, flags=flags),
    )(xt, w, mean, var, g, b)
    return jnp.transpose(out, (2, 0, 1))
  return f
pallas_standalone__batchnorm__sampling_kernel = jax.jit(make(sep=False, U=2))
```

```python
import jax
import jax.numpy as jnp
from jax.experimental import pallas as pl
from jax.experimental.pallas import tpu as pltpu

P, Q = 0.5, 2.0
P2, Q2 = P * P, Q * Q
N0 = P2 * Q2
NP = 2 * P2 * (P2 - Q2)
NQ = 2 * Q2 * (Q2 - P2)
U = 2
D = 3
RX = 8
RO = 4
BF, F32 = jnp.bfloat16, jnp.float32


def _kernel(x_hbm, w_hbm, mean_ref, var_ref, g_ref, b_ref, o_hbm,
            e_ref, wbuf, xbuf, obuf, u_ref, sc_ref, sh_ref, sem_w, sem_x, sem_o):
    S, C, B = x_hbm.shape
    assert S == 32 and B % 128 == 0
    NJ = S // 4
    T = (B // 128) * NJ
    KT = (C + 127) // 128
    rows = [min(128, C - kt * 128) for kt in range(KT)]

    def hbm_tile(ref, t):
        return ref.at[pl.ds(4 * (t & 7), 4), :,
                      pl.ds(pl.multiple_of((t >> 3) * 128, 128), 128)]

    def x_dma(t):
        sl = t & (RX - 1)
        return pltpu.make_async_copy(hbm_tile(x_hbm, t), xbuf.at[sl], sem_x.at[sl])

    def o_dma(t):
        sl = t & (RO - 1)
        return pltpu.make_async_copy(obuf.at[sl], hbm_tile(o_hbm, t), sem_o.at[sl])

    wds = [pltpu.make_async_copy(w_hbm.at[:, pl.ds(kt * 128, rows[kt]), :],
                                 wbuf.at[:, pl.ds(kt * 128, rows[kt]), :],
                                 sem_w.at[kt]) for kt in range(KT)]
    for d in wds:
        d.start()
    for t in range(2):
        x_dma(t).start()
    xbuf[RX - 1, 3] = jnp.zeros((C, 128), BF)
    inv = 1.0 / jnp.sqrt(var_ref[...].astype(F32) + 1e-5)
    sc = (g_ref[...].astype(F32) * inv).reshape(1, C)
    sh = b_ref[...].astype(F32).reshape(1, C) - mean_ref[...].astype(F32).reshape(1, C) * sc
    sc_ref[...] = jnp.broadcast_to(sc * 0.5, (128, C)).T
    sh_ref[...] = jnp.broadcast_to(sh * 0.5, (128, C)).T
    for kt in range(KT):
        wds[kt].wait()
        nr = rows[kt]
        scv = sc_ref[:, :nr]
        w0, w1, w2 = [wbuf[k, pl.ds(kt * 128, nr), :].T.astype(F32) * scv for k in range(3)]
        a, c = w0 + P2 * w2, w0 + Q2 * w2
        us = [w0 * (1.0 / N0), (a + P * w1) * (1.0 / NP), (a - P * w1) * (1.0 / NP),
              (c + Q * w1) * (1.0 / NQ), (c - Q * w1) * (1.0 / NQ), w2]
        for i in range(6):
            u_ref[i, kt, :, :nr] = us[i].astype(BF)
    for t in range(2, 1 + D):
        x_dma(t).start()
    x_dma(0).wait()

    def first_rhs(t):
        cur = t & (RX - 1)
        d1, d2, d3, d4 = [xbuf[cur, i].astype(F32) for i in range(4)]
        return ((d4 - Q2 * d2) + P * (d3 - Q2 * d1)).astype(BF)

    def compute(t, carried):
        j = t & 7
        cur = t & (RX - 1)
        d1, d2, d3, d4 = [xbuf[cur, i].astype(F32) for i in range(4)]
        d0 = jnp.where(j > 0, xbuf[(t + RX - 1) & (RX - 1), 3].astype(F32), 0.0)
        d5 = jnp.where(j < NJ - 1, xbuf[(t + 1) & (RX - 1), 0].astype(F32), 0.0)

        def dot(i, e):
            lhs = jnp.concatenate([u_ref[i, kt][:, :rows[kt]] for kt in range(KT)], axis=1)
            return jnp.dot(lhs, e.astype(BF), preferred_element_type=F32)

        shv = sh_ref[...]

        def fin(i, y):
            h = y + shv
            obuf[t & (RO - 1), i] = (h * jnp.tanh(h) + h).astype(BF)

        ea, eb = d4 - Q2 * d2, P * (d3 - Q2 * d1)
        m1 = dot(1, e_ref[...] if carried else ea + eb)
        m2 = dot(2, ea - eb)
        s1, t1 = m1 + m2, m1 - m2
        ec, ed = d4 - P2 * d2, Q * (d3 - P2 * d1)
        m3 = dot(3, ec + ed)
        m4 = dot(4, ec - ed)
        s2, t2 = m3 + m4, m3 - m4
        m0 = dot(0, N0 * d0 - (P2 + Q2) * d2 + d4)
        fin(1, P * t1 + Q * t2)
        fin(2, P2 * s1 + Q2 * s2)
        m5 = dot(5, N0 * d1 - (P2 + Q2) * d3 + d5)
        fin(0, m0 + s1 + s2)
        fin(3, P2 * P * t1 + Q2 * Q * t2 + m5)

    def body(it, _):
        t0 = it * U
        for k in range(U):
            t = t0 + k

            @pl.when(t + 1 < T)
            def _():
                sl = (t + 1) & (RX - 1)
                pltpu.make_async_copy(xbuf.at[sl], xbuf.at[sl], sem_x.at[sl]).wait()

            @pl.when(t >= RO)
            def _():
                sl = t & (RO - 1)
                pltpu.make_async_copy(obuf.at[sl], obuf.at[sl], sem_o.at[sl]).wait()
        for k in range(U):
            t = t0 + k
            if k == U - 1:
                nxt = first_rhs(t0 + U)
            compute(t, k == 0)
            if k == U - 1:
                e_ref[...] = nxt
            o_dma(t).start()

            @pl.when(t + 1 + D < T)
            def _():
                x_dma(t + 1 + D).start()
        return 0

    e_ref[...] = first_rhs(0)
    jax.lax.fori_loop(0, T // U, body, 0)
    for t in range(T - RO, T):
        o_dma(t).wait()


@jax.jit
def pallas_standalone__batchnorm__sampling_kernel(x, w, mean, var, g, b):
    B, S, C = x.shape
    KT = (C + 127) // 128
    vm = pl.BlockSpec(memory_space=pltpu.VMEM)
    hbm = pl.BlockSpec(memory_space=pl.ANY)
    out = pl.pallas_call(
        _kernel,
        in_specs=[hbm, hbm, vm, vm, vm, vm],
        out_specs=hbm,
        out_shape=jax.ShapeDtypeStruct((S, C, B), x.dtype),
        scratch_shapes=[
            pltpu.VMEM((C, 128), BF),
            pltpu.VMEM((3, C, C), BF),
            pltpu.VMEM((RX, 4, C, 128), BF),
            pltpu.VMEM((RO, 4, C, 128), BF),
            pltpu.VMEM((6, KT, C, 128), BF),
            pltpu.VMEM((C, 128), F32),
            pltpu.VMEM((C, 128), F32),
            pltpu.SemaphoreType.DMA((KT,)),
            pltpu.SemaphoreType.DMA((RX,)),
            pltpu.SemaphoreType.DMA((RO,)),
        ],
        compiler_params=pltpu.CompilerParams(vmem_limit_bytes=64 * 1024 * 1024),
    )(jnp.transpose(x, (1, 2, 0)), w, mean, var, g, b)
    return jnp.transpose(out, (2, 0, 1))
```
